```python
import os as _os
_os.environ.setdefault("JAX_PLATFORMS", "cpu")
import jax
import jax.numpy as jnp

def _softmax(x, axis=-1):
    return jax.nn.softmax(x, axis=axis)
def _gelu(x):
    return jax.nn.gelu(x, approximate=True)
def _silu(x):
    return jax.nn.silu(x)
def _sigmoid(x):
    return jax.nn.sigmoid(x)
def _layernorm(x, axis=-1, eps=1e-5):
    m = jnp.mean(x, axis=axis, keepdims=True)
    v = jnp.var(x, axis=axis, keepdims=True)
    return (x - m) / jnp.sqrt(v + eps)
def _scatter_add(tgt, idx, src, axis=0):
    return tgt.at[idx].add(src)
def _segment_sum(src, seg, n):
    return jax.ops.segment_sum(src, seg, n)
class _Rng:
    def __init__(self, key):
        self._k = key
    def _next(self):
        self._k, sub = jax.random.split(self._k)
        return sub
    def normal(self, shape):
        return jax.random.normal(self._next(), shape, dtype=jnp.bfloat16)
    def randint(self, lo, hi, shape):
        return jax.random.randint(self._next(), shape, lo, hi, dtype=jnp.int32)
    def uniform(self, shape, lo=0.0, hi=1.0):
        return jax.random.uniform(self._next(), shape, jnp.bfloat16, lo, hi)
    def permutation(self, n):
        return jax.random.permutation(self._next(), n)


kernel_name = 'standalone__mha_softmax__near_ridge'

def setup_inputs():
    _rng = _Rng(jax.random.key(int.from_bytes(__import__("os").urandom(4), "little")))
    _w = (lambda a: (lambda t: t.astype(jnp.bfloat16) if jnp.issubdtype(t.dtype, jnp.floating) else t)(jnp.asarray(a)))
    B, H, Sq, Sk, D = 8, 16, 192, 1024, 256
    return {
        "q": _w((lambda *s: _rng.normal(s) * 0.4)(B, H, Sq, D)),
        "k": _w((lambda *s: _rng.normal(s) * 0.4)(B, H, Sk, D)),
        "v": _w((lambda *s: _rng.normal(s) * 0.05)(B, H, Sk, D)),
    }

def reference(q, k, v):
    scale = q.shape[-1] ** -0.5
    scores = jnp.einsum("bhqd,bhkd->bhqk", q, k) * scale
    p = _softmax(scores, axis=-1)
    return jnp.einsum("bhqk,bhkd->bhqd", p, v)
```

```python
import math

import jax
import jax.numpy as jnp
from jax import lax
import jax.experimental.pallas as pl
import jax.experimental.pallas.tpu as pltpu

_GROUP = 8
_AHEAD = 11
_SLOTS = 3
_READ_HEADS = 2
_KV_ROWS = 32
_Q_ROWS = 64
_OUT_ROWS = 32
_OUT_DELAY = 2
_OUT_FIRST = 6


def _attention_kernel(q_hbm, k_hbm, v_hbm, o_hbm,
                      q_buf, kv_buf, o_buf, in_sems, out_sem):
  _, num_groups, seq_q, head_dim = q_hbm.shape
  seq_k = k_hbm.shape[2]
  num_slices = _GROUP * num_groups
  slice_rows = seq_k // _GROUP
  first_q_part = _GROUP - seq_q // _Q_ROWS
  exp2_scale = head_dim ** -0.5 * math.log2(math.e)
  q_sem = in_sems.at[2]

  def row_slice(start, size):
    if not isinstance(start, int):
      start = pl.multiple_of(start, size)
    return pl.ds(start, size)

  def start_slice(index, _=None):
    group, part = index // _GROUP, index % _GROUP
    slot = group % _SLOTS

    @pl.when(part >= first_q_part)
    def _():
      rows = row_slice((part - first_q_part) * _Q_ROWS, _Q_ROWS)
      for n, head in enumerate(range(0, _GROUP, _READ_HEADS)):
        heads = pl.ds(head, _READ_HEADS)
        pltpu.make_async_copy(
            q_hbm.at[heads, group, rows], q_buf.at[slot, heads, rows], q_sem
        ).start(priority=n % 2)

    for row in range(0, slice_rows, _KV_ROWS):
      rows = row_slice(part * slice_rows + row, _KV_ROWS)
      for head in range(0, _GROUP, _READ_HEADS):
        for n, src in enumerate((k_hbm, v_hbm)):
          heads = pl.ds((head + n * _GROUP // 2) % _GROUP, _READ_HEADS)
          pltpu.make_async_copy(
              src.at[heads, group, rows], kv_buf.at[slot, n, heads, rows],
              in_sems.at[group % 2]
          ).start(priority=n)

  def wait_q(group):
    buf = q_buf.at[group % _SLOTS]
    pltpu.make_async_copy(buf, buf, q_sem).wait()

  def wait_kv(group):
    buf = kv_buf.at[group % _SLOTS]
    pltpu.make_async_copy(buf, buf, in_sems.at[group % 2]).wait()

  def start_write(group, _=None):
    for row in range(0, seq_q, _OUT_ROWS):
      block = (slice(None), group, pl.ds(row, _OUT_ROWS))
      pltpu.make_async_copy(
          o_buf.at[block], o_hbm.at[block], out_sem).start(priority=1)

  def attend(group, head):
    slot = group % _SLOTS
    q = q_buf[slot, head]
    k = kv_buf[slot, 0, head]
    v = kv_buf[slot, 1, head]
    s = lax.dot_general(q, k, (((1,), (1,)), ((), ())),
                        preferred_element_type=jnp.float32)
    m = jnp.max(s, axis=-1, keepdims=True)
    p = jnp.exp2((s - m) * exp2_scale)
    l = jnp.sum(p, axis=-1, keepdims=True)
    o = jnp.dot(p.astype(v.dtype), v, preferred_element_type=jnp.float32)
    o_buf[head, group] = (o * (1.0 / l)).astype(o_buf.dtype)

  start_slice(0)
  lax.fori_loop(1, _AHEAD, start_slice, None)

  first_write = num_slices - 1 + _OUT_DELAY

  def group_body(group, _):
    @pl.when(group < num_groups - 1)
    def _():
      wait_q(group)

    wait_kv(group)

    def head_body(head, _):
      index = group * _GROUP + head + _AHEAD

      @pl.when(index < num_slices)
      def _():
        start_slice(index)

      @pl.when(index == first_write)
      def _():
        wait_q(num_groups - 1)
        lax.fori_loop(0, _OUT_FIRST, start_write, None)

      @pl.when(index > first_write)
      def _():
        start_write(_OUT_FIRST - 1 + index - first_write)

      attend(group, head)

    lax.fori_loop(0, _GROUP, head_body, None)

  lax.fori_loop(0, num_groups, group_body, None)
  lax.fori_loop(_OUT_FIRST + _AHEAD - _OUT_DELAY, num_groups, start_write, None)
  pltpu.make_async_copy(o_buf, o_hbm, out_sem).wait()


@jax.jit
def pallas_standalone__mha_softmax__near_ridge_kernel(
    q: jax.Array,
    k: jax.Array,
    v: jax.Array,
):
  batch, heads, seq_q, head_dim = q.shape
  seq_k = k.shape[2]
  num_heads = batch * heads
  num_groups = num_heads // _GROUP
  assert num_heads % _GROUP == 0 and seq_k % (_GROUP * _KV_ROWS) == 0
  assert seq_q % _Q_ROWS == 0 and seq_q % _OUT_ROWS == 0
  assert _GROUP - 1 <= _AHEAD <= (_SLOTS - 1) * _GROUP and _AHEAD <= 2 * _GROUP
  assert _GROUP - seq_q // _Q_ROWS >= max(_AHEAD - _GROUP, 0)
  assert 1 <= _OUT_DELAY <= _AHEAD - _GROUP + 1
  for step in range(_OUT_DELAY - 1, _AHEAD):
    written = _OUT_FIRST + step - (_OUT_DELAY - 1)
    assert written <= (num_heads - _AHEAD + step) // _GROUP

  def grouped(x):
    return x.reshape(_GROUP, num_groups, *x.shape[2:])

  out = pl.pallas_call(
      _attention_kernel,
      in_specs=[pl.BlockSpec(memory_space=pl.ANY)] * 3,
      out_specs=pl.BlockSpec(memory_space=pl.ANY),
      out_shape=jax.ShapeDtypeStruct(
          (_GROUP, num_groups, seq_q, head_dim), q.dtype),
      scratch_shapes=[
          pltpu.VMEM((_SLOTS, _GROUP, seq_q, head_dim), q.dtype),
          pltpu.VMEM((_SLOTS, 2, _GROUP, seq_k, head_dim), k.dtype),
          pltpu.VMEM((_GROUP, num_groups, seq_q, head_dim), q.dtype),
          pltpu.SemaphoreType.DMA((3,)),
          pltpu.SemaphoreType.DMA(()),
      ],
      compiler_params=pltpu.CompilerParams(
          vmem_limit_bytes=64 * 1024 * 1024,
          disable_bounds_checks=True,
      ),
  )(grouped(q), grouped(k), grouped(v))
  return out.reshape(batch, heads, seq_q, head_dim)
```
